```python
import os as _os
_os.environ.setdefault("JAX_PLATFORMS", "cpu")
import jax
import jax.numpy as jnp

def _softmax(x, axis=-1):
    return jax.nn.softmax(x, axis=axis)
def _gelu(x):
    return jax.nn.gelu(x, approximate=True)
def _silu(x):
    return jax.nn.silu(x)
def _sigmoid(x):
    return jax.nn.sigmoid(x)
def _layernorm(x, axis=-1, eps=1e-5):
    m = jnp.mean(x, axis=axis, keepdims=True)
    v = jnp.var(x, axis=axis, keepdims=True)
    return (x - m) / jnp.sqrt(v + eps)
def _scatter_add(tgt, idx, src, axis=0):
    return tgt.at[idx].add(src)
def _segment_sum(src, seg, n):
    return jax.ops.segment_sum(src, seg, n)
class _Rng:
    def __init__(self, key):
        self._k = key
    def _next(self):
        self._k, sub = jax.random.split(self._k)
        return sub
    def normal(self, shape):
        return jax.random.normal(self._next(), shape, dtype=jnp.bfloat16)
    def randint(self, lo, hi, shape):
        return jax.random.randint(self._next(), shape, lo, hi, dtype=jnp.int32)
    def uniform(self, shape, lo=0.0, hi=1.0):
        return jax.random.uniform(self._next(), shape, jnp.bfloat16, lo, hi)
    def permutation(self, n):
        return jax.random.permutation(self._next(), n)


kernel_name = 'concat_heads__sliding_local_dilated__sliding_block__prompt'

def setup_inputs():
    _rng = _Rng(jax.random.key(int.from_bytes(__import__("os").urandom(4), "little")))
    _w = (lambda a: (lambda t: t.astype(jnp.bfloat16) if jnp.issubdtype(t.dtype, jnp.floating) else t)(jnp.asarray(a)))
    def _A_setup():
        B, S, D = 1, 2048, 1024
        return {
            "x": _w((lambda *s: _rng.normal(s) * 0.2)(B, S, D)),
            "wqkv": _w((lambda *s: _rng.normal(s) * 0.2)(D, 3 * D)),
            "wo": _w((lambda *s: _rng.normal(s) * 0.05)(D, D)),
        }
    _A_in = _A_setup()

    def _B_setup():
        B, S, D = 1, 2048, 1024
        return {
            "x": _w((lambda *s: _rng.normal(s) * 0.2)(B, S, D)),
            "wqkv": _w((lambda *s: _rng.normal(s) * 0.2)(D, 3 * D)),
            "wo": _w((lambda *s: _rng.normal(s) * 0.05)(D, D)),
        }
    _B_in = _B_setup()

    return {
        "A_x": _A_in["x"],
        "A_wqkv": _A_in["wqkv"],
        "A_wo": _A_in["wo"],
        "B_x": _B_in["x"],
        "B_wqkv": _B_in["wqkv"],
        "B_wo": _B_in["wo"],
    }

def reference(A_x, A_wqkv, A_wo, B_x, B_wqkv, B_wo):
    def _A_ref(x, wqkv, wo):
        B, S, D = x.shape
        H = 32; Dh = D // H
        W, dil = 8, 2
        qkv = (lambda x, *d: x.transpose(*d))((x @ wqkv).reshape(B, S, 3, H, Dh), 2, 0, 3, 1, 4)
        q, k, v = qkv[0], qkv[1], qkv[2]
        scale = Dh ** -0.5
        pos = jnp.arange(S)
        off = jnp.arange(W) * dil
        idx = pos[:, None] - off[None, :]
        mask = idx >= 0
        idx_c = jnp.where(mask, idx, 0).reshape(-1)
        kg = k[:, :, idx_c, :].reshape(B, H, S, W, Dh)
        vg = v[:, :, idx_c, :].reshape(B, H, S, W, Dh)
        logits = jnp.einsum("bhsd,bhswd->bhsw", q, kg) * scale
        logits = jnp.where(mask[None, None, :, :], logits, -1e9)
        attn = _softmax(logits, axis=-1)
        o = jnp.einsum("bhsw,bhswd->bhsd", attn, vg)
        return (lambda x, *d: x.transpose(*d))(o, 0, 2, 1, 3).reshape(B, S, D) @ wo

    def _B_ref(x, wqkv, wo):
        B, S, D = x.shape
        H = 32; Dh = D // H; W = 256
        qkv = (lambda x, *d: x.transpose(*d))((x @ wqkv).reshape(B, S, 3, H, Dh), 2, 0, 3, 1, 4)
        q, k, v = qkv[0], qkv[1], qkv[2]
        scores = jnp.einsum("bhqd,bhkd->bhqk", q, k) * (Dh ** -0.5)
        idx = jnp.arange(S)
        mask = (idx[:, None] - idx[None, :] >= 0) & (idx[:, None] - idx[None, :] < W)
        scores = jnp.where(mask[None, None], scores, -1e9)
        p = _softmax(scores, axis=-1)
        o = jnp.einsum("bhqk,bhkd->bhqd", p, v)
        return (lambda x, *d: x.transpose(*d))(o, 0, 2, 1, 3).reshape(B, S, D) @ wo

    a = _A_ref(A_x, A_wqkv, A_wo)
    b = _B_ref(B_x, B_wqkv, B_wo)
    return jnp.concatenate([a, b], axis=-1)
```

```python
import os
import jax
import jax.numpy as jnp
import jax.experimental.pallas as pl
import jax.experimental.pallas.tpu as pltpu

S, D, H, DH = 2048, 1024, 32, 32
TQ = 256
QB = 128
WB = 256
WA, DIL = 8, 2
HA = 16
NG = D // 128
LOG2E = 1.4426950408889634
SCALE = DH ** -0.5 * LOG2E
NEG = -1e9
KW = WB + QB
KA = HA + QB
VAR = TQ + QB
NSB = TQ // QB
NSTEP = S // TQ
NT = (((1,), (1,)), ((), ()))
NW = int(os.environ.get("NW", 512))


def _kernel(ax_ref, awqkv_hbm, awo_hbm, bx_ref, bwqkv_hbm, bwo_hbm, o_ref,
            ka_scr, va_scr, kb_scr, vbt_scr, s_scr, bias_scr, sa_scr, biasa_scr, vat_scr, qb_scr, oa_scr,
            awqkv_ref, awo_ref, bwqkv_ref, bwo_ref, sems):
    i = pl.program_id(0)
    f32, bf16 = jnp.float32, jnp.bfloat16
    row0 = pl.multiple_of(i * TQ, TQ)

    def cols(g):
        return slice(128 * g, 128 * (g + 1))

    def wcopy(k):
        if k < 3:
            return pltpu.make_async_copy(awqkv_hbm.at[:, k * D:(k + 1) * D], awqkv_ref.at[:, k * D:(k + 1) * D], sems.at[k])
        src_, dst_ = [(bwqkv_hbm, bwqkv_ref), (awo_hbm, awo_ref), (bwo_hbm, bwo_ref)][k - 3]
        return pltpu.make_async_copy(src_, dst_, sems.at[k])

    def wait0(k):
        @pl.when(i == 0)
        def _():
            wcopy(k).wait()

    @pl.when(i == 0)
    def _():
        for k in range(6):
            wcopy(k).start()
        ka_scr[0:HA, :] = jnp.zeros((HA, D), bf16)
        va_scr[...] = jnp.zeros((VAR, D), f32)
        kb_scr[0:WB, :] = jnp.zeros((WB, D), bf16)
        vbt_scr[:, 0:WB] = jnp.zeros((D, WB), bf16)

    r = jax.lax.broadcasted_iota(jnp.int32, (KW, QB), 1)
    c = jax.lax.broadcasted_iota(jnp.int32, (KW, QB), 0)
    band = (c > r) & (c <= r + WB)
    ra = jax.lax.broadcasted_iota(jnp.int32, (KA, QB), 1)
    ca = jax.lax.broadcasted_iota(jnp.int32, (KA, QB), 0) - HA
    dlt = ra - ca
    banda = (dlt >= 0) & (dlt < WA * DIL) & (dlt % DIL == 0)
    for sb in range(NSB):
        bias_scr[sb] = jnp.where(band & (c + (row0 + sb * QB) >= WB), 0.0, NEG).astype(f32)
        biasa_scr[sb] = jnp.where(banda & (ca + (row0 + sb * QB) >= 0), 0.0, NEG).astype(f32)

    wait0(0)
    qa = (jnp.dot(ax_ref[...], awqkv_ref[:, :D], preferred_element_type=f32).astype(bf16).astype(f32) * SCALE).astype(bf16)
    wait0(1)
    ka_scr[HA:HA + TQ, :] = jnp.dot(ax_ref[...], awqkv_ref[:, D:2 * D], preferred_element_type=f32).astype(bf16)
    wait0(2)
    va_scr[HA:HA + TQ, :] = jnp.dot(ax_ref[...], awqkv_ref[:, 2 * D:], preferred_element_type=f32)
    vat_scr[...] = va_scr[...].T.astype(bf16)

    def projb_tasks():
        ts = []
        for c0 in range(0, 3 * D, NW):
            def f(c0=c0):
                y = jnp.dot(bx_ref[...], bwqkv_ref[:, c0:c0 + NW], preferred_element_type=f32)
                if c0 < D:
                    qb_scr[:, c0:c0 + NW] = (y.astype(bf16).astype(f32) * SCALE).astype(bf16)
                elif c0 < 2 * D:
                    kb_scr[pl.ds(WB + row0, TQ), c0 - D:c0 - D + NW] = y.astype(bf16)
                else:
                    vbt_scr[c0 - 2 * D:c0 - 2 * D + NW, pl.ds(WB + row0, TQ)] = y.T.astype(bf16)
            ts.append(f)
        return ts

    def outa_tasks():
        ts = []
        for c0 in range(0, D, NW):
            def f(c0=c0):
                o_ref[:, c0:c0 + NW] = jnp.dot(oa_scr[...], awo_ref[:, c0:c0 + NW], preferred_element_type=f32).astype(o_ref.dtype)
            ts.append(f)
        return ts

    lane_head = jax.lax.broadcasted_iota(jnp.int32, (QB, 128), 1) // DH

    def stack_heads(qg):
        return jnp.concatenate([jnp.where(lane_head == j, qg, jnp.zeros_like(qg)) for j in range(4)], axis=0)

    chains = [(sb, g) for g in range(NG) for sb in range(NSB)]

    def qk_b(n):
        sb, g = chains[n]
        start = pl.multiple_of(row0 + sb * QB, QB)
        qst = stack_heads(qb_scr[sb * QB:(sb + 1) * QB, cols(g)])
        s_scr[n % 2] = jax.lax.dot_general(kb_scr[pl.ds(start, KW), cols(g)], qst, NT, preferred_element_type=f32)

    def qk_a(n):
        sb, g = chains[n]
        qst = stack_heads(qa[sb * QB:(sb + 1) * QB, cols(g)])
        sa_scr[n % 2] = jax.lax.dot_general(ka_scr[sb * QB:sb * QB + KA, cols(g)], qst, NT, preferred_element_type=f32)

    def head_out(s, vt):
        mx = jnp.max(s, axis=0, keepdims=True)
        p = jnp.exp2(s - mx)
        den = jnp.sum(p, axis=0, keepdims=True)
        return jnp.dot(vt, p.astype(bf16), preferred_element_type=f32) * (1.0 / den)

    def rest_b(n):
        sb, g = chains[n]
        start = pl.multiple_of(row0 + sb * QB, QB)
        outs = []
        for j in range(4):
            s = s_scr[n % 2, :, j * QB:(j + 1) * QB] + bias_scr[sb]
            outs.append(head_out(s, vbt_scr[128 * g + DH * j:128 * g + DH * (j + 1), pl.ds(start, KW)]))
        return jnp.concatenate(outs, axis=0).T.astype(bf16)

    def rest_a(n):
        sb, g = chains[n]
        outs = []
        for j in range(4):
            s = sa_scr[n % 2, :, j * QB:(j + 1) * QB] + biasa_scr[sb]
            outs.append(head_out(s, vat_scr[128 * g + DH * j:128 * g + DH * (j + 1), sb * QB:sb * QB + KA]))
        return jnp.concatenate(outs, axis=0).T.astype(bf16)

    wait0(3)
    tasks = projb_tasks()
    nch = len(chains)
    qk_a(0)
    done = 0
    for n in range(nch):
        if n + 1 < nch:
            qk_a(n + 1)
        sb, g = chains[n]
        oa_scr[sb * QB:(sb + 1) * QB, cols(g)] = rest_a(n)
        while done < (n + 1) * len(tasks) // nch:
            tasks[done](); done += 1
    ka_scr[0:HA, :] = ka_scr[TQ:TQ + HA, :]
    va_scr[0:HA, :] = va_scr[TQ:TQ + HA, :]

    wait0(4)
    tasks = outa_tasks()
    ob = {}
    qk_b(0)
    done = 0
    for n in range(nch):
        if n + 1 < nch:
            qk_b(n + 1)
        ob[chains[n]] = rest_b(n)
        while done < (n + 1) * len(tasks) // nch:
            tasks[done](); done += 1
    obf = jnp.concatenate([jnp.concatenate([ob[(sb, g)] for g in range(NG)], axis=1) for sb in range(NSB)], axis=0)
    wait0(5)
    o_ref[:, D:] = jnp.dot(obf, bwo_ref[...], preferred_element_type=f32).astype(o_ref.dtype)


@jax.jit
def pallas_concat_heads__sliding_local_dilated__sliding_block__prompt_kernel(A_x, A_wqkv, A_wo, B_x, B_wqkv, B_wo):
    ax = A_x.reshape(S, D)
    bx = B_x.reshape(S, D)
    full = lambda shp: pl.BlockSpec(memory_space=pl.ANY)
    cur = pl.BlockSpec((TQ, D), lambda i: (i, 0))
    out = pl.pallas_call(
        _kernel,
        grid=(NSTEP,),
        in_specs=[cur, full((D, 3 * D)), full((D, D)), cur, full((D, 3 * D)), full((D, D))],
        out_specs=pl.BlockSpec((TQ, 2 * D), lambda i: (i, 0)),
        out_shape=jax.ShapeDtypeStruct((S, 2 * D), jnp.bfloat16),
        scratch_shapes=[
            pltpu.VMEM((TQ + HA, D), jnp.bfloat16),
            pltpu.VMEM((VAR, D), jnp.float32),
            pltpu.VMEM((S + WB, D), jnp.bfloat16),
            pltpu.VMEM((D, S + WB), jnp.bfloat16),
            pltpu.VMEM((2, KW, 4 * QB), jnp.float32),
            pltpu.VMEM((NSB, KW, QB), jnp.float32),
            pltpu.VMEM((2, KA, 4 * QB), jnp.float32),
            pltpu.VMEM((NSB, KA, QB), jnp.float32),
            pltpu.VMEM((D, VAR), jnp.bfloat16),
            pltpu.VMEM((TQ, D), jnp.bfloat16),
            pltpu.VMEM((TQ, D), jnp.bfloat16),
            pltpu.VMEM((D, 3 * D), jnp.bfloat16),
            pltpu.VMEM((D, D), jnp.bfloat16),
            pltpu.VMEM((D, 3 * D), jnp.bfloat16),
            pltpu.VMEM((D, D), jnp.bfloat16),
            pltpu.SemaphoreType.DMA((6,)),
        ],
        compiler_params=pltpu.CompilerParams(
            dimension_semantics=("arbitrary",),
            vmem_limit_bytes=100 * 1024 * 1024,
        ),
    )(ax, A_wqkv, A_wo, bx, B_wqkv, B_wo)
    return out.reshape(1, S, 2 * D)
```

```python
import jax
import jax.numpy as jnp
import jax.experimental.pallas as pl
import jax.experimental.pallas.tpu as pltpu

S, D, H, DH = 2048, 1024, 32, 32
TQ = 256
QB = 128
WB = 256
WA, DIL = 8, 2
HA = 16
NG = D // 128
LOG2E = 1.4426950408889634
SCALE = DH ** -0.5 * LOG2E
NEG = -1e9
KW = WB + QB
KA = HA + QB
VAR = TQ + QB
NSB = TQ // QB
NSTEP = S // TQ
NT = (((1,), (1,)), ((), ()))
NW = 512


def _kernel(ax_ref, awqkv_hbm, awo_hbm, bx_ref, bwqkv_hbm, bwo_hbm, o_ref,
            ka_scr, va_scr, kb_scr, vbt_scr, s_scr, bias_scr, sa_scr, biasa_scr, vat_scr, qb_scr, oa_scr,
            awqkv_ref, awo_ref, bwqkv_ref, bwo_ref, sems):
    i = pl.program_id(0)
    f32, bf16 = jnp.float32, jnp.bfloat16
    row0 = pl.multiple_of(i * TQ, TQ)

    def cols(g):
        return slice(128 * g, 128 * (g + 1))

    def wcopy(k):
        if k < 3:
            return pltpu.make_async_copy(awqkv_hbm.at[:, k * D:(k + 1) * D], awqkv_ref.at[:, k * D:(k + 1) * D],
                                         sems.at[k])
        src_, dst_ = [(bwqkv_hbm, bwqkv_ref), (awo_hbm, awo_ref), (bwo_hbm, bwo_ref)][k - 3]
        return pltpu.make_async_copy(src_, dst_, sems.at[k])

    def wait0(ks):
        @pl.when(i == 0)
        def _():
            for k in ks:
                wcopy(k).wait()

    @pl.when(i == 0)
    def _():
        for k in range(6):
            wcopy(k).start()
        ka_scr[0:HA, :] = jnp.zeros((HA, D), bf16)
        va_scr[...] = jnp.zeros((VAR, D), f32)
        kb_scr[0:WB, :] = jnp.zeros((WB, D), bf16)
        vbt_scr[:, 0:WB] = jnp.zeros((D, WB), bf16)

    @pl.when(i <= 1)
    def _():
        r = jax.lax.broadcasted_iota(jnp.int32, (KW, QB), 1)
        c = jax.lax.broadcasted_iota(jnp.int32, (KW, QB), 0)
        band = (c > r) & (c <= r + WB)
        ra = jax.lax.broadcasted_iota(jnp.int32, (KA, QB), 1)
        ca = jax.lax.broadcasted_iota(jnp.int32, (KA, QB), 0) - HA
        dlt = ra - ca
        banda = (dlt >= 0) & (dlt < WA * DIL) & (dlt % DIL == 0)
        for sb in range(NSB):
            bias_scr[sb] = jnp.where(band & (c + (row0 + sb * QB) >= WB), 0.0, NEG).astype(f32)
            biasa_scr[sb] = jnp.where(banda & (ca + (row0 + sb * QB) >= 0), 0.0, NEG).astype(f32)

    wait0((0, 1, 2))
    qa = (jnp.dot(ax_ref[...], awqkv_ref[:, :D], preferred_element_type=f32).astype(bf16).astype(f32)
          * SCALE).astype(bf16)
    ka_scr[HA:HA + TQ, :] = jnp.dot(ax_ref[...], awqkv_ref[:, D:2 * D], preferred_element_type=f32).astype(bf16)
    va_scr[HA:HA + TQ, :] = jnp.dot(ax_ref[...], awqkv_ref[:, 2 * D:], preferred_element_type=f32)
    vat_scr[...] = va_scr[...].T.astype(bf16)

    def projb_tasks():
        ts = []
        for c0 in range(0, 3 * D, NW):
            def f(c0=c0):
                y = jnp.dot(bx_ref[...], bwqkv_ref[:, c0:c0 + NW], preferred_element_type=f32)
                if c0 < D:
                    qb_scr[:, c0:c0 + NW] = (y.astype(bf16).astype(f32) * SCALE).astype(bf16)
                elif c0 < 2 * D:
                    kb_scr[pl.ds(WB + row0, TQ), c0 - D:c0 - D + NW] = y.astype(bf16)
                else:
                    vbt_scr[c0 - 2 * D:c0 - 2 * D + NW, pl.ds(WB + row0, TQ)] = y.T.astype(bf16)
            ts.append(f)
        return ts

    def outa_tasks():
        ts = []
        for c0 in range(0, D, NW):
            def f(c0=c0):
                o_ref[:, c0:c0 + NW] = jnp.dot(oa_scr[...], awo_ref[:, c0:c0 + NW],
                                               preferred_element_type=f32).astype(o_ref.dtype)
            ts.append(f)
        return ts

    lane_head = jax.lax.broadcasted_iota(jnp.int32, (QB, 128), 1) // DH

    def stack_heads(qg):
        return jnp.concatenate([jnp.where(lane_head == j, qg, jnp.zeros_like(qg)) for j in range(4)], axis=0)

    chains = [(sb, g) for g in range(NG) for sb in range(NSB)]

    def qk_b(n):
        sb, g = chains[n]
        start = pl.multiple_of(row0 + sb * QB, QB)
        qst = stack_heads(qb_scr[sb * QB:(sb + 1) * QB, cols(g)])
        s_scr[n % 2] = jax.lax.dot_general(kb_scr[pl.ds(start, KW), cols(g)], qst, NT, preferred_element_type=f32)

    def qk_a(n):
        sb, g = chains[n]
        qst = stack_heads(qa[sb * QB:(sb + 1) * QB, cols(g)])
        sa_scr[n % 2] = jax.lax.dot_general(ka_scr[sb * QB:sb * QB + KA, cols(g)], qst, NT,
                                            preferred_element_type=f32)

    def head_out(s, vt):
        mx = jnp.max(s, axis=0, keepdims=True)
        p = jnp.exp2(s - mx)
        den = jnp.sum(p, axis=0, keepdims=True)
        return jnp.dot(vt, p.astype(bf16), preferred_element_type=f32) * (1.0 / den)

    def rest_b(n):
        sb, g = chains[n]
        start = pl.multiple_of(row0 + sb * QB, QB)
        outs = []
        for j in range(4):
            s = s_scr[n % 2, :, j * QB:(j + 1) * QB] + bias_scr[sb]
            outs.append(head_out(s, vbt_scr[128 * g + DH * j:128 * g + DH * (j + 1), pl.ds(start, KW)]))
        return jnp.concatenate(outs, axis=0).T.astype(bf16)

    def rest_a(n):
        sb, g = chains[n]
        outs = []
        for j in range(4):
            s = sa_scr[n % 2, :, j * QB:(j + 1) * QB] + biasa_scr[sb]
            outs.append(head_out(s, vat_scr[128 * g + DH * j:128 * g + DH * (j + 1), sb * QB:sb * QB + KA]))
        return jnp.concatenate(outs, axis=0).T.astype(bf16)

    nch = len(chains)

    wait0((3,))
    tasks = projb_tasks()
    qk_a(0)
    done = 0
    for n in range(nch):
        if n + 1 < nch:
            qk_a(n + 1)
        sb, g = chains[n]
        oa_scr[sb * QB:(sb + 1) * QB, cols(g)] = rest_a(n)
        while done < (n + 1) * len(tasks) // nch:
            tasks[done]()
            done += 1
    ka_scr[0:HA, :] = ka_scr[TQ:TQ + HA, :]
    va_scr[0:HA, :] = va_scr[TQ:TQ + HA, :]

    wait0((4, 5))
    tasks = outa_tasks()
    ob = {}
    qk_b(0)
    done = 0
    for n in range(nch):
        if n + 1 < nch:
            qk_b(n + 1)
        ob[chains[n]] = rest_b(n)
        while done < (n + 1) * len(tasks) // nch:
            tasks[done]()
            done += 1

    obf = jnp.concatenate([jnp.concatenate([ob[(sb, g)] for g in range(NG)], axis=1) for sb in range(NSB)], axis=0)
    o_ref[:, D:] = jnp.dot(obf, bwo_ref[...], preferred_element_type=f32).astype(o_ref.dtype)


@jax.jit
def pallas_concat_heads__sliding_local_dilated__sliding_block__prompt_kernel(
    A_x: jax.Array,
    A_wqkv: jax.Array,
    A_wo: jax.Array,
    B_x: jax.Array,
    B_wqkv: jax.Array,
    B_wo: jax.Array,
):
    ax = A_x.reshape(S, D)
    bx = B_x.reshape(S, D)
    hbm = pl.BlockSpec(memory_space=pl.ANY)
    rows = pl.BlockSpec((TQ, D), lambda i: (i, 0))
    out = pl.pallas_call(
        _kernel,
        grid=(NSTEP,),
        in_specs=[rows, hbm, hbm, rows, hbm, hbm],
        out_specs=pl.BlockSpec((TQ, 2 * D), lambda i: (i, 0)),
        out_shape=jax.ShapeDtypeStruct((S, 2 * D), jnp.bfloat16),
        scratch_shapes=[
            pltpu.VMEM((TQ + HA, D), jnp.bfloat16),
            pltpu.VMEM((VAR, D), jnp.float32),
            pltpu.VMEM((S + WB, D), jnp.bfloat16),
            pltpu.VMEM((D, S + WB), jnp.bfloat16),
            pltpu.VMEM((2, KW, 4 * QB), jnp.float32),
            pltpu.VMEM((NSB, KW, QB), jnp.float32),
            pltpu.VMEM((2, KA, 4 * QB), jnp.float32),
            pltpu.VMEM((NSB, KA, QB), jnp.float32),
            pltpu.VMEM((D, VAR), jnp.bfloat16),
            pltpu.VMEM((TQ, D), jnp.bfloat16),
            pltpu.VMEM((TQ, D), jnp.bfloat16),
            pltpu.VMEM((D, 3 * D), jnp.bfloat16),
            pltpu.VMEM((D, D), jnp.bfloat16),
            pltpu.VMEM((D, 3 * D), jnp.bfloat16),
            pltpu.VMEM((D, D), jnp.bfloat16),
            pltpu.SemaphoreType.DMA((6,)),
        ],
        compiler_params=pltpu.CompilerParams(
            dimension_semantics=("arbitrary",),
            vmem_limit_bytes=100 * 1024 * 1024,
        ),
    )(ax, A_wqkv, A_wo, bx, B_wqkv, B_wo)
    return out.reshape(1, S, 2 * D)
```

```python
import jax
import jax.numpy as jnp
import jax.experimental.pallas as pl
import jax.experimental.pallas.tpu as pltpu

S, D, H, DH = 2048, 1024, 32, 32
TQ = 256
QB = 128
QA = 64
WB = 256
WA, DIL = 8, 2
HA = 16
NG = D // 128
LOG2E = 1.4426950408889634
SCALE = DH ** -0.5 * LOG2E
NEG = -1e9
KW = WB + QB
KA = HA + QA
VAR = TQ + 128
NSB = TQ // QB
NSQ = TQ // QA
NSTEP = S // TQ
NT = (((1,), (1,)), ((), ()))
LA = 8
LAA = 8
NSL, NSA = LA + 1, LAA + 1
NWF = 128
NWO = 512


def _kernel(ax_ref, awqkv_hbm, awo_hbm, bx_ref, bwqkv_hbm, bwo_hbm, o_ref,
            ka_scr, va_scr, kb_scr, vbt_scr, s_scr, bias_scr, sa_scr, biasa_scr, vat_scr, qa_scr, ob_scr,
            awqkv_ref, awo_ref, bwqkv_ref, bwo_ref, sems):
    i = pl.program_id(0)
    f32, bf16 = jnp.float32, jnp.bfloat16
    row0 = pl.multiple_of(i * TQ, TQ)

    def cols(g):
        return slice(128 * g, 128 * (g + 1))

    def wcopy(k):
        if k < 3:
            return pltpu.make_async_copy(bwqkv_hbm.at[:, k * D:(k + 1) * D], bwqkv_ref.at[:, k * D:(k + 1) * D],
                                         sems.at[k])
        src_, dst_ = [(awqkv_hbm, awqkv_ref), (bwo_hbm, bwo_ref), (awo_hbm, awo_ref)][k - 3]
        return pltpu.make_async_copy(src_, dst_, sems.at[k])

    def wait0(ks):
        @pl.when(i == 0)
        def _():
            for k in ks:
                wcopy(k).wait()

    @pl.when(i == 0)
    def _():
        for k in range(6):
            wcopy(k).start()
        ka_scr[0:HA, :] = jnp.zeros((HA, D), bf16)
        va_scr[...] = jnp.zeros((VAR, D), f32)
        kb_scr[0:WB, :] = jnp.zeros((WB, D), bf16)
        vbt_scr[:, 0:WB] = jnp.zeros((D, WB), bf16)

    @pl.when(i <= 1)
    def _():
        r = jax.lax.broadcasted_iota(jnp.int32, (KW, QB), 1)
        c = jax.lax.broadcasted_iota(jnp.int32, (KW, QB), 0)
        band = (c > r) & (c <= r + WB)
        ra = jax.lax.broadcasted_iota(jnp.int32, (KA, 128), 1) % QA
        ca = jax.lax.broadcasted_iota(jnp.int32, (KA, 128), 0) - HA
        dlt = ra - ca
        banda = (dlt >= 0) & (dlt < WA * DIL) & (dlt % DIL == 0)
        for sb in range(2):
            bias_scr[sb] = jnp.where(band & (c + (row0 + sb * QB) >= WB), 0.0, NEG).astype(f32)
            biasa_scr[sb] = jnp.where(banda & (ca + (row0 + sb * QA) >= 0), 0.0, NEG).astype(f32)

    wait0((0, 1, 2))
    vbt_scr[:, pl.ds(WB + row0, TQ)] = jnp.dot(bx_ref[...], bwqkv_ref[:, 2 * D:],
                                               preferred_element_type=f32).T.astype(bf16)
    kb_scr[pl.ds(WB + row0, TQ), :] = jnp.dot(bx_ref[...], bwqkv_ref[:, D:2 * D],
                                              preferred_element_type=f32).astype(bf16)
    qb = (jnp.dot(bx_ref[...], bwqkv_ref[:, :D], preferred_element_type=f32).astype(bf16).astype(f32)
          * SCALE).astype(bf16)

    def proja_tasks():
        ts = []
        for c0 in list(range(2 * D, 3 * D, NWF)) + list(range(D, 2 * D, NWF)) + list(range(0, D, NWF)):
            def f(c0=c0):
                y = jnp.dot(ax_ref[...], awqkv_ref[:, c0:c0 + NWF], preferred_element_type=f32)
                if c0 < D:
                    qa_scr[:, c0:c0 + NWF] = (y.astype(bf16).astype(f32) * SCALE).astype(bf16)
                elif c0 < 2 * D:
                    ka_scr[HA:HA + TQ, c0 - D:c0 - D + NWF] = y.astype(bf16)
                else:
                    c1 = c0 - 2 * D
                    va_scr[HA:HA + TQ, c1:c1 + NWF] = y
                    vat_scr[c1:c1 + NWF, :] = va_scr[:, c1:c1 + NWF].T.astype(bf16)
            ts.append(f)
        return ts

    def outb_tasks():
        ts = []
        for c0 in range(0, D, NWO):
            def f(c0=c0):
                o_ref[:, D + c0:D + c0 + NWO] = jnp.dot(ob_scr[...], bwo_ref[:, c0:c0 + NWO],
                                                        preferred_element_type=f32).astype(o_ref.dtype)
            ts.append(f)
        return ts

    chains = [(sb, g) for g in range(NG) for sb in range(NSB)]
    lane_head = jax.lax.broadcasted_iota(jnp.int32, (QB, 128), 1) // DH

    def qk_b(h):
        n, j = h // 4, h % 4
        sb, g = chains[n]
        start = pl.multiple_of(row0 + sb * QB, QB)
        qg = qb[sb * QB:(sb + 1) * QB, cols(g)]
        qm = jnp.where(lane_head == j, qg, jnp.zeros_like(qg))
        s_scr[h % NSL] = jax.lax.dot_general(
            kb_scr[pl.ds(start, KW), cols(g)], qm, NT, preferred_element_type=f32) + bias_scr[sb]

    chains_a = [(sq, g) for g in range(NG) for sq in range(NSQ)]
    lane_head_a = jax.lax.broadcasted_iota(jnp.int32, (QA, 128), 1) // DH

    def qk_a(n):
        sq, g = chains_a[n]
        qg = qa_scr[sq * QA:(sq + 1) * QA, cols(g)]
        qst = jnp.concatenate([jnp.where(lane_head_a == j, qg, jnp.zeros_like(qg)) for j in range(4)], axis=0)
        sa_scr[n % NSA] = jax.lax.dot_general(ka_scr[sq * QA:sq * QA + KA, cols(g)], qst, NT,
                                              preferred_element_type=f32)

    def head_out(s, vt):
        mx = jnp.max(s, axis=0, keepdims=True)
        p = jnp.exp2(s - mx)
        den = jnp.sum(p, axis=0, keepdims=True)
        return jnp.dot(vt, p.astype(bf16), preferred_element_type=f32) * (1.0 / den)

    def rest_b(h):
        n, j = h // 4, h % 4
        sb, g = chains[n]
        start = pl.multiple_of(row0 + sb * QB, QB)
        return head_out(s_scr[h % NSL], vbt_scr[128 * g + DH * j:128 * g + DH * (j + 1), pl.ds(start, KW)])

    def rest_a(n):
        sq, g = chains_a[n]
        outs = []
        for u in range(2):
            s = sa_scr[n % NSA, :, u * 128:(u + 1) * 128] + biasa_scr[min(sq, 1)]
            outs.append(head_out(s, vat_scr[128 * g + 64 * u:128 * g + 64 * (u + 1), sq * QA:sq * QA + KA]))
        return outs

    lane_lo = jax.lax.broadcasted_iota(jnp.int32, (DH, 128), 1) < QA

    def merge_a(e, f):
        rows = []
        for u in range(2):
            rows.append(jnp.where(lane_lo, e[u][:DH], pltpu.roll(f[u][:DH], QA, 1)))
            rows.append(jnp.where(lane_lo, pltpu.roll(e[u][DH:], QA, 1), f[u][DH:]))
        return jnp.concatenate(rows, axis=0).T.astype(bf16)

    wait0((3,))
    tasks = proja_tasks()
    nh = 4 * len(chains)
    for h in range(LA):
        qk_b(h)
    done = 0
    for n in range(len(chains)):
        outs = []
        for j in range(4):
            h = 4 * n + j
            if h + LA < nh:
                qk_b(h + LA)
            outs.append(rest_b(h))
            while done < min(len(tasks), (h + 4) * len(tasks) // (nh + 3)):
                tasks[done]()
                done += 1
        sb, g = chains[n]
        ob_scr[sb * QB:(sb + 1) * QB, cols(g)] = jnp.concatenate(outs, axis=0).T.astype(bf16)

    wait0((4, 5))
    tasks = outb_tasks()
    ncha = len(chains_a)
    for n in range(LAA):
        qk_a(n)
    done = 0
    prev = None
    oa = {}
    for n in range(ncha):
        if n + LAA < ncha:
            qk_a(n + LAA)
        sq, g = chains_a[n]
        cur = rest_a(n)
        if sq % 2 == 1:
            oa[(sq // 2, g)] = merge_a(prev, cur)
        prev = cur
        while done < (n + 1) * len(tasks) // ncha:
            tasks[done]()
            done += 1
    ka_scr[0:HA, :] = ka_scr[TQ:TQ + HA, :]
    va_scr[0:HA, :] = va_scr[TQ:TQ + HA, :]

    oaf = jnp.concatenate([jnp.concatenate([oa[(sb, g)] for g in range(NG)], axis=1) for sb in range(NSB)], axis=0)
    o_ref[:, :D] = jnp.dot(oaf, awo_ref[...], preferred_element_type=f32).astype(o_ref.dtype)


@jax.jit
def pallas_concat_heads__sliding_local_dilated__sliding_block__prompt_kernel(
    A_x: jax.Array,
    A_wqkv: jax.Array,
    A_wo: jax.Array,
    B_x: jax.Array,
    B_wqkv: jax.Array,
    B_wo: jax.Array,
):
    ax = A_x.reshape(S, D)
    bx = B_x.reshape(S, D)
    hbm = pl.BlockSpec(memory_space=pl.ANY)
    rows = pl.BlockSpec((TQ, D), lambda i: (i, 0))
    out = pl.pallas_call(
        _kernel,
        grid=(NSTEP,),
        in_specs=[rows, hbm, hbm, rows, hbm, hbm],
        out_specs=pl.BlockSpec((TQ, 2 * D), lambda i: (i, 0)),
        out_shape=jax.ShapeDtypeStruct((S, 2 * D), jnp.bfloat16),
        scratch_shapes=[
            pltpu.VMEM((TQ + HA, D), jnp.bfloat16),
            pltpu.VMEM((VAR, D), jnp.float32),
            pltpu.VMEM((S + WB, D), jnp.bfloat16),
            pltpu.VMEM((D, S + WB), jnp.bfloat16),
            pltpu.VMEM((NSL, KW, QB), jnp.float32),
            pltpu.VMEM((2, KW, QB), jnp.float32),
            pltpu.VMEM((NSA, KA, 4 * QA), jnp.float32),
            pltpu.VMEM((2, KA, 128), jnp.float32),
            pltpu.VMEM((D, VAR), jnp.bfloat16),
            pltpu.VMEM((TQ, D), jnp.bfloat16),
            pltpu.VMEM((TQ, D), jnp.bfloat16),
            pltpu.VMEM((D, 3 * D), jnp.bfloat16),
            pltpu.VMEM((D, D), jnp.bfloat16),
            pltpu.VMEM((D, 3 * D), jnp.bfloat16),
            pltpu.VMEM((D, D), jnp.bfloat16),
            pltpu.SemaphoreType.DMA((6,)),
        ],
        compiler_params=pltpu.CompilerParams(
            dimension_semantics=("arbitrary",),
            vmem_limit_bytes=100 * 1024 * 1024,
        ),
    )(ax, A_wqkv, A_wo, bx, B_wqkv, B_wo)
    return out.reshape(1, S, 2 * D)
```
